```python
import os as _os
_os.environ.setdefault("JAX_PLATFORMS", "cpu")
import jax
import jax.numpy as jnp

def _softmax(x, axis=-1):
    return jax.nn.softmax(x, axis=axis)
def _gelu(x):
    return jax.nn.gelu(x, approximate=True)
def _silu(x):
    return jax.nn.silu(x)
def _sigmoid(x):
    return jax.nn.sigmoid(x)
def _layernorm(x, axis=-1, eps=1e-5):
    m = jnp.mean(x, axis=axis, keepdims=True)
    v = jnp.var(x, axis=axis, keepdims=True)
    return (x - m) / jnp.sqrt(v + eps)
def _scatter_add(tgt, idx, src, axis=0):
    return tgt.at[idx].add(src)
def _segment_sum(src, seg, n):
    return jax.ops.segment_sum(src, seg, n)
class _Rng:
    def __init__(self, key):
        self._k = key
    def _next(self):
        self._k, sub = jax.random.split(self._k)
        return sub
    def normal(self, shape):
        return jax.random.normal(self._next(), shape, dtype=jnp.bfloat16)
    def randint(self, lo, hi, shape):
        return jax.random.randint(self._next(), shape, lo, hi, dtype=jnp.int32)
    def uniform(self, shape, lo=0.0, hi=1.0):
        return jax.random.uniform(self._next(), shape, jnp.bfloat16, lo, hi)
    def permutation(self, n):
        return jax.random.permutation(self._next(), n)


kernel_name = 'gated_mix__ssm_conv_s5__glu_gated_geglu__prompt'

def setup_inputs():
    _rng = _Rng(jax.random.key(int.from_bytes(__import__("os").urandom(4), "little")))
    _w = (lambda a: (lambda t: t.astype(jnp.bfloat16) if jnp.issubdtype(t.dtype, jnp.floating) else t)(jnp.asarray(a)))
    def _A_setup():
        B, S, D = 1, 2048, 448
        P = D
        Lambda_re = -0.5 * jnp.exp((lambda *s: _rng.normal(s) * 0.4)(P))
        Lambda_im = (lambda *s: _rng.normal(s) * 0.4)(P) * 1.0
        B_re = (lambda *s: _rng.normal(s) * 0.4)(P, D) * (D ** -0.5)
        B_im = (lambda *s: _rng.normal(s) * 0.4)(P, D) * (D ** -0.5)
        C_re = (lambda *s: _rng.normal(s) * 0.4)(D, P) * (P ** -0.5)
        C_im = (lambda *s: _rng.normal(s) * 0.4)(D, P) * (P ** -0.5)
        log_dt = (lambda *s: _rng.normal(s) * 0.4)(P) * 0.3 - 2.0
        Dskip = (lambda *s: _rng.normal(s) * 0.4)(D)
        return {
            "x": _w((lambda *s: _rng.normal(s) * 0.05)(B, S, D)),
            "Lambda_re": _w(Lambda_re),
            "Lambda_im": _w(Lambda_im),
            "B_re": _w(B_re),
            "B_im": _w(B_im),
            "C_re": _w(C_re),
            "C_im": _w(C_im),
            "log_dt": _w(log_dt),
            "Dskip": _w(Dskip),
        }
    _A_in = _A_setup()

    def _B_setup():
        B, S, Dm, Df = 1, 2048, 448, 1792
        return {
            "x": _w((lambda *s: _rng.normal(s) * 0.05)(B, S, Dm)),
            "w_gate": _w((lambda *s: _rng.normal(s) * 1.6)(Dm, Df) * (Dm ** -0.5)),
            "w_up": _w((lambda *s: _rng.normal(s) * 1.6)(Dm, Df) * (Dm ** -0.5)),
            "w_down": _w((lambda *s: _rng.normal(s) * 1.6)(Df, Dm) * (Df ** -0.5)),
        }
    _B_in = _B_setup()

    return {
        "A_x": _A_in["x"],
        "A_Lambda_re": _A_in["Lambda_re"],
        "A_Lambda_im": _A_in["Lambda_im"],
        "A_B_re": _A_in["B_re"],
        "A_B_im": _A_in["B_im"],
        "A_C_re": _A_in["C_re"],
        "A_C_im": _A_in["C_im"],
        "A_log_dt": _A_in["log_dt"],
        "A_Dskip": _A_in["Dskip"],
        "B_x": _B_in["x"],
        "B_w_gate": _B_in["w_gate"],
        "B_w_up": _B_in["w_up"],
        "B_w_down": _B_in["w_down"],
        "gate_w": _w((lambda *s: _rng.normal(s) * 0.05)(448) * 16.0),
    }

def reference(A_x, A_Lambda_re, A_Lambda_im, A_B_re, A_B_im, A_C_re, A_C_im, A_log_dt, A_Dskip, B_x, B_w_gate, B_w_up, B_w_down, gate_w):
    def _A_ref(x, Lambda_re, Lambda_im, B_re, B_im, C_re, C_im, log_dt, Dskip):
        Bsz, L, H = x.shape
        Lam = Lambda_re + 1j * Lambda_im
        Bmat = B_re + 1j * B_im
        Cmat = C_re + 1j * C_im
        dt = jnp.exp(log_dt)
        Lam_bar = jnp.exp(dt * Lam)
        B_bar = ((Lam_bar - 1.0) / Lam)[:, None] * Bmat
        Bu = jnp.einsum("bld,pd->blp", x + 0j, B_bar)
        h = jnp.zeros_like(Bu[:, 0, :])
        hs = []
        for t in range(L):
            h = Lam_bar[None, :] * h + Bu[:, t, :]
            hs.append(h)
        hseq = jnp.stack(hs, 1)
        y = 2.0 * jnp.einsum("blp,dp->bld", hseq, Cmat).real + x * Dskip[None, None, :]
        return y

    def _B_ref(x, w_gate, w_up, w_down):
        g = jnp.einsum("bsd,df->bsf", x, w_gate)
        u = jnp.einsum("bsd,df->bsf", x, w_up)
        h = _gelu(g) * u
        return jnp.einsum("bsf,fd->bsd", h, w_down)

    x = A_x
    g = _sigmoid((x * gate_w).sum(-1, keepdims=True))
    a = _A_ref(x, A_Lambda_re, A_Lambda_im, A_B_re, A_B_im, A_C_re, A_C_im, A_log_dt, A_Dskip)
    b = _B_ref(x, B_w_gate, B_w_up, B_w_down)
    return g * a + (1 - g) * b
```

```python
import functools
import math

import jax
import jax.numpy as jnp
import jax.experimental.pallas as pl
import jax.experimental.pallas.tpu as pltpu

_F32 = jnp.float32
_BF16 = jnp.bfloat16


def _rb(v):
    return v.astype(_BF16).astype(_F32)


def _dot(a, b):
    return jax.lax.dot_general(a, b, (((1,), (0,)), ((), ())),
                               preferred_element_type=_F32)


def _dot_t(a, b):
    return jax.lax.dot_general(a, b, (((1,), (1,)), ((), ())),
                               preferred_element_type=_F32)


def _ssm_glu_kernel(
    x_ref,
    wg_ref,
    wu_ref,
    wd_ref,
    bre_ref,
    bim_ref,
    cre_ref,
    cim_ref,
    lre_ref,
    lim_ref,
    ldt_ref,
    dskip_ref,
    gw_ref,
    o_ref,
    tab_ref,
    car_ref,
    *,
    T: int,
    NPOW: int,
):
    c = pl.program_id(0)
    D = x_ref.shape[1]
    P = lre_ref.shape[1]

    @pl.when(c == 0)
    def _init():
        lr = lre_ref[...].astype(_F32)
        li = lim_ref[...].astype(_F32)
        dt = jnp.exp(ldt_ref[...]).astype(_F32)
        ar = dt * lr
        ai = dt * li
        er = jnp.exp(ar)
        lbr = er * jnp.cos(ai)
        lbi = er * jnp.sin(ai)
        nr = lbr - 1.0
        ni = lbi
        den = lr * lr + li * li
        qr = (nr * lr + ni * li) / den
        qi = (ni * lr - nr * li) / den
        kk = jnp.left_shift(
            jnp.int32(1),
            jax.lax.broadcasted_iota(jnp.int32, (NPOW, 1), 0)).astype(_F32)
        akr = kk * ar
        aki = kk * ai
        ek = jnp.exp(akr)
        tab_ref[0:NPOW, :] = ek * jnp.cos(aki)
        tab_ref[NPOW:2 * NPOW, :] = ek * jnp.sin(aki)
        tab_ref[2 * NPOW:2 * NPOW + 1, :] = qr
        tab_ref[2 * NPOW + 1:2 * NPOW + 2, :] = qi
        tab_ref[2 * NPOW + 2:2 * NPOW + 3, :] = lbr
        tab_ref[2 * NPOW + 3:2 * NPOW + 4, :] = lbi
        car_ref[...] = jnp.zeros_like(car_ref)

    x = x_ref[...]

    prod = x * gw_ref[...]
    s = jnp.sum(prod.astype(_F32), axis=-1, keepdims=True)
    s = _rb(s)
    gate = _rb(1.0 / (1.0 + jnp.exp(-s)))
    omg = _rb(1.0 - gate)

    g = _dot(x, wg_ref[...])
    u = _dot(x, wu_ref[...])
    g = _rb(g)
    u = _rb(u)
    gg = jax.nn.gelu(g, approximate=True)
    hf = (gg * u).astype(_BF16)
    b = _dot(hf, wd_ref[...])
    b = _rb(b)

    wr = _dot_t(x, bre_ref[...])
    wi = _dot_t(x, bim_ref[...])
    qr = tab_ref[2 * NPOW:2 * NPOW + 1, :]
    qi = tab_ref[2 * NPOW + 1:2 * NPOW + 2, :]
    vr = wr * qr - wi * qi
    vi = wr * qi + wi * qr

    lbr = tab_ref[2 * NPOW + 2:2 * NPOW + 3, :]
    lbi = tab_ref[2 * NPOW + 3:2 * NPOW + 4, :]
    cr = car_ref[0:1, :]
    ci = car_ref[8:9, :]
    injr = lbr * cr - lbi * ci
    inji = lbr * ci + lbi * cr
    rows = jax.lax.broadcasted_iota(jnp.int32, (T, P), 0)
    first = rows == 0
    vr = jnp.where(first, vr + injr, vr)
    vi = jnp.where(first, vi + inji, vi)

    k = 1
    j = 0
    while k < T:
        lkr = tab_ref[j:j + 1, :]
        lki = tab_ref[NPOW + j:NPOW + j + 1, :]
        sr = pltpu.roll(vr, k, axis=0)
        si = pltpu.roll(vi, k, axis=0)
        keep = rows >= k
        sr = jnp.where(keep, sr, 0.0)
        si = jnp.where(keep, si, 0.0)
        vr, vi = vr + lkr * sr - lki * si, vi + lkr * si + lki * sr
        k *= 2
        j += 1

    car_ref[0:1, :] = vr[T - 1:T, :]
    car_ref[8:9, :] = vi[T - 1:T, :]

    y = _dot_t(vr.astype(_BF16), cre_ref[...]) - _dot_t(vi.astype(_BF16), cim_ref[...])
    skip = (x * dskip_ref[...]).astype(_F32)
    a = 2.0 * y + skip

    o_ref[...] = gate * a + _rb(omg * b)


@jax.jit
def pallas_gated_mix__ssm_conv_s5__glu_gated_geglu__prompt_kernel(
    A_x: jax.Array,
    A_Lambda_re: jax.Array,
    A_Lambda_im: jax.Array,
    A_B_re: jax.Array,
    A_B_im: jax.Array,
    A_C_re: jax.Array,
    A_C_im: jax.Array,
    A_log_dt: jax.Array,
    A_Dskip: jax.Array,
    B_x: jax.Array,
    B_w_gate: jax.Array,
    B_w_up: jax.Array,
    B_w_down: jax.Array,
    gate_w: jax.Array,
):
    Bsz, L, D = A_x.shape
    P = A_Lambda_re.shape[0]
    F = B_w_gate.shape[1]
    T = 256
    assert L % T == 0
    NPOW = int(math.log2(T))

    x2 = A_x.reshape(Bsz * L, D)
    lre = A_Lambda_re.reshape(1, P)
    lim = A_Lambda_im.reshape(1, P)
    ldt = A_log_dt.reshape(1, P)
    dskip = A_Dskip.reshape(1, D)
    gw = gate_w.reshape(1, D)

    nchunks = (Bsz * L) // T
    kernel = functools.partial(_ssm_glu_kernel, T=T, NPOW=NPOW)

    const = lambda shape: pl.BlockSpec(shape, lambda c: tuple(0 for _ in shape))

    out = pl.pallas_call(
        kernel,
        grid=(nchunks,),
        in_specs=[
            pl.BlockSpec((T, D), lambda c: (c, 0)),
            const((D, F)),
            const((D, F)),
            const((F, D)),
            const((P, D)),
            const((P, D)),
            const((D, P)),
            const((D, P)),
            const((1, P)),
            const((1, P)),
            const((1, P)),
            const((1, D)),
            const((1, D)),
        ],
        out_specs=pl.BlockSpec((T, D), lambda c: (c, 0)),
        out_shape=jax.ShapeDtypeStruct((Bsz * L, D), _F32),
        scratch_shapes=[
            pltpu.VMEM((2 * NPOW + 4, P), _F32),
            pltpu.VMEM((16, P), _F32),
        ],
        compiler_params=pltpu.CompilerParams(
            dimension_semantics=("arbitrary",),
            vmem_limit_bytes=100 * 1024 * 1024,
        ),
    )(x2, B_w_gate, B_w_up, B_w_down, A_B_re, A_B_im, A_C_re, A_C_im,
      lre, lim, ldt, dskip, gw)
    return out.reshape(Bsz, L, D)
```

```python
import functools

import jax
import jax.numpy as jnp
import jax.experimental.pallas as pl
import jax.experimental.pallas.tpu as pltpu

_F32 = jnp.float32
_BF16 = jnp.bfloat16
_G = 8


def _rb(v):
    return v.astype(_BF16).astype(_F32)


def _dot(a, b):
    return jax.lax.dot_general(a, b, (((1,), (0,)), ((), ())),
                               preferred_element_type=_F32)


def _dot_t(a, b):
    return jax.lax.dot_general(a, b, (((1,), (1,)), ((), ())),
                               preferred_element_type=_F32)


_TAB_L = 0
_TAB_P8 = 48
_TAB_Q = 64
_TAB_ROWS = 72


def _ssm_glu_kernel(
    x_ref,
    wg_ref,
    wu_ref,
    wdt_ref,
    bre_ref,
    bim_ref,
    cre_ref,
    cim_ref,
    lre_ref,
    lim_ref,
    ldt_ref,
    dskip_ref,
    gw_ref,
    o_ref,
    tab_ref,
    car_ref,
    *,
    T: int,
    FS: int,
):
    c = pl.program_id(0)
    D = x_ref.shape[0]
    P = lre_ref.shape[0]
    F = wg_ref.shape[1]
    NSLAB = F // FS
    NGRP = T // _G

    @pl.when(c == 0)
    def _init():
        lr = lre_ref[...].reshape(1, P).astype(_F32)
        li = lim_ref[...].reshape(1, P).astype(_F32)
        dt = jnp.exp(ldt_ref[...].reshape(1, P)).astype(_F32)
        ar = dt * lr
        ai = dt * li
        er = jnp.exp(ar)
        lbr = er * jnp.cos(ai)
        lbi = er * jnp.sin(ai)
        nr = lbr - 1.0
        ni = lbi
        den = lr * lr + li * li
        qr = (nr * lr + ni * li) / den
        qi = (ni * lr - nr * li) / den
        tab_ref[_TAB_Q:_TAB_Q + 1, :] = qr
        tab_ref[_TAB_Q + 1:_TAB_Q + 2, :] = qi
        rowi = jax.lax.broadcasted_iota(jnp.int32, (_G, P), 0)
        rowf = rowi.astype(_F32)
        for s, k in enumerate((1, 2, 4)):
            ek = jnp.exp(float(k) * ar)
            lkr = ek * jnp.cos(float(k) * ai)
            lki = ek * jnp.sin(float(k) * ai)
            keep = rowi >= k
            tab_ref[_TAB_L + 16 * s:_TAB_L + 16 * s + 8, :] = jnp.where(keep, lkr, 0.0)
            tab_ref[_TAB_L + 16 * s + 8:_TAB_L + 16 * s + 16, :] = jnp.where(keep, lki, 0.0)
        kk = rowf + 1.0
        ek = jnp.exp(kk * ar)
        tab_ref[_TAB_P8:_TAB_P8 + 8, :] = ek * jnp.cos(kk * ai)
        tab_ref[_TAB_P8 + 8:_TAB_P8 + 16, :] = ek * jnp.sin(kk * ai)
        car_ref[...] = jnp.zeros_like(car_ref)

    x = x_ref[...].T

    wr = _dot_t(x, bre_ref[...])
    wi = _dot_t(x, bim_ref[...])
    qr = tab_ref[_TAB_Q:_TAB_Q + 1, :]
    qi = tab_ref[_TAB_Q + 1:_TAB_Q + 2, :]
    vr = wr * qr - wi * qi
    vi = wr * qi + wi * qr

    prod = x * gw_ref[...].reshape(1, D)
    s = jnp.sum(prod.astype(_F32), axis=-1, keepdims=True)
    s = _rb(s)
    gate = _rb(1.0 / (1.0 + jnp.exp(-s)))
    omg = _rb(1.0 - gate)

    def ffn_slab(j):
        wgs = wg_ref[:, j * FS:(j + 1) * FS]
        wus = wu_ref[:, j * FS:(j + 1) * FS]
        g = _rb(_dot(x, wgs))
        u = _rb(_dot(x, wus))
        gg = jax.nn.gelu(g, approximate=True)
        hf = (gg * u).astype(_BF16)
        wds = wdt_ref[:, j * FS:(j + 1) * FS]
        return _dot_t(hf, wds)

    b = None
    j = 0

    for s, k in enumerate((1, 2, 4)):
        if j < NSLAB:
            bj = ffn_slab(j)
            b = bj if b is None else b + bj
            j += 1
        lkr = tab_ref[_TAB_L + 16 * s:_TAB_L + 16 * s + 8, :]
        lki = tab_ref[_TAB_L + 16 * s + 8:_TAB_L + 16 * s + 16, :]
        sr3 = pltpu.roll(vr, k, axis=0).reshape(NGRP, _G, P)
        si3 = pltpu.roll(vi, k, axis=0).reshape(NGRP, _G, P)
        vr3 = vr.reshape(NGRP, _G, P)
        vi3 = vi.reshape(NGRP, _G, P)
        vr = (vr3 + lkr[None] * sr3 - lki[None] * si3).reshape(T, P)
        vi = (vi3 + lkr[None] * si3 + lki[None] * sr3).reshape(T, P)

    while j < NSLAB:
        bj = ffn_slab(j)
        b = bj if b is None else b + bj
        j += 1
    b = _rb(b)

    p8r = tab_ref[_TAB_P8:_TAB_P8 + 8, :]
    p8i = tab_ref[_TAB_P8 + 8:_TAB_P8 + 16, :]
    cr = car_ref[0:1, :]
    ci = car_ref[8:9, :]
    vr3 = vr.reshape(NGRP, _G, P)
    vi3 = vi.reshape(NGRP, _G, P)
    out_r = []
    out_i = []
    for g in range(NGRP):
        cbr = jnp.broadcast_to(cr, (_G, P))
        cbi = jnp.broadcast_to(ci, (_G, P))
        gr = vr3[g] + (p8r * cbr - p8i * cbi)
        gi = vi3[g] + (p8r * cbi + p8i * cbr)
        out_r.append(gr)
        out_i.append(gi)
        cr = gr[_G - 1:_G, :]
        ci = gi[_G - 1:_G, :]
    car_ref[0:1, :] = cr
    car_ref[8:9, :] = ci
    vr = jnp.concatenate(out_r, axis=0)
    vi = jnp.concatenate(out_i, axis=0)

    y = (_dot_t(vr.astype(_BF16), cre_ref[...])
         - _dot_t(vi.astype(_BF16), cim_ref[...]))
    skip = (x * dskip_ref[...].reshape(1, D)).astype(_F32)
    a = 2.0 * y + skip

    o_ref[...] = (gate * a + _rb(omg * b)).T


@jax.jit
def pallas_gated_mix__ssm_conv_s5__glu_gated_geglu__prompt_kernel(
    A_x: jax.Array,
    A_Lambda_re: jax.Array,
    A_Lambda_im: jax.Array,
    A_B_re: jax.Array,
    A_B_im: jax.Array,
    A_C_re: jax.Array,
    A_C_im: jax.Array,
    A_log_dt: jax.Array,
    A_Dskip: jax.Array,
    B_x: jax.Array,
    B_w_gate: jax.Array,
    B_w_up: jax.Array,
    B_w_down: jax.Array,
    gate_w: jax.Array,
):
    Bsz, L, D = A_x.shape
    P = A_Lambda_re.shape[0]
    F = B_w_gate.shape[1]
    T = 256
    FS = 256
    assert L % T == 0 and F % FS == 0 and T % _G == 0
    nchunks = (Bsz * L) // T

    xT = A_x.reshape(Bsz * L, D).T
    wdt = B_w_down.T

    kernel = functools.partial(_ssm_glu_kernel, T=T, FS=FS)

    def const(shape):
        return pl.BlockSpec(shape, lambda c: tuple(0 for _ in shape))

    outT = pl.pallas_call(
        kernel,
        grid=(nchunks,),
        in_specs=[
            pl.BlockSpec((D, T), lambda c: (0, c)),
            const((D, F)),
            const((D, F)),
            const((D, F)),
            const((P, D)),
            const((P, D)),
            const((D, P)),
            const((D, P)),
            const((P,)),
            const((P,)),
            const((P,)),
            const((D,)),
            const((D,)),
        ],
        out_specs=pl.BlockSpec((D, T), lambda c: (0, c)),
        out_shape=jax.ShapeDtypeStruct((D, Bsz * L), _F32),
        scratch_shapes=[
            pltpu.VMEM((_TAB_ROWS, P), _F32),
            pltpu.VMEM((16, P), _F32),
        ],
        compiler_params=pltpu.CompilerParams(
            dimension_semantics=("arbitrary",),
            vmem_limit_bytes=100 * 1024 * 1024,
        ),
    )(xT, B_w_gate, B_w_up, wdt, A_B_re, A_B_im, A_C_re, A_C_im,
      A_Lambda_re, A_Lambda_im, A_log_dt, A_Dskip, gate_w)
    return outT.T.reshape(Bsz, L, D)
```

```python
import functools

import jax
import jax.numpy as jnp
import jax.experimental.pallas as pl
import jax.experimental.pallas.tpu as pltpu

_F32 = jnp.float32
_BF16 = jnp.bfloat16
_G = 8


def _rb(v):
    return v.astype(_BF16).astype(_F32)


def _dot(a, b):
    return jax.lax.dot_general(a, b, (((1,), (0,)), ((), ())),
                               preferred_element_type=_F32)


def _dot_t(a, b):
    return jax.lax.dot_general(a, b, (((1,), (1,)), ((), ())),
                               preferred_element_type=_F32)


_TAB_L = 0
_TAB_P8 = 48
_TAB_Q = 64
_TAB_ROWS = 72


def _ssm_glu_kernel(
    x_ref,
    wg_ref,
    wu_ref,
    wdt_ref,
    bre_ref,
    bim_ref,
    cre_ref,
    cim_ref,
    lre_ref,
    lim_ref,
    ldt_ref,
    dskip_ref,
    gw_ref,
    o_ref,
    tab_ref,
    car_ref,
    *,
    T: int,
    FS: int,
):
    c = pl.program_id(0)
    D = x_ref.shape[0]
    P = lre_ref.shape[0]
    F = wg_ref.shape[1]
    NSLAB = F // FS
    NGRP = T // _G

    @pl.when(c == 0)
    def _init():
        lr = lre_ref[...].reshape(1, P).astype(_F32)
        li = lim_ref[...].reshape(1, P).astype(_F32)
        dt = jnp.exp(ldt_ref[...].reshape(1, P)).astype(_F32)
        ar = dt * lr
        ai = dt * li
        er = jnp.exp(ar)
        lbr = er * jnp.cos(ai)
        lbi = er * jnp.sin(ai)
        nr = lbr - 1.0
        ni = lbi
        den = lr * lr + li * li
        qr = (nr * lr + ni * li) / den
        qi = (ni * lr - nr * li) / den
        tab_ref[_TAB_Q:_TAB_Q + 1, :] = qr
        tab_ref[_TAB_Q + 1:_TAB_Q + 2, :] = qi
        rowi = jax.lax.broadcasted_iota(jnp.int32, (_G, P), 0)
        rowf = rowi.astype(_F32)
        for s, k in enumerate((1, 2, 4)):
            ek = jnp.exp(float(k) * ar)
            lkr = ek * jnp.cos(float(k) * ai)
            lki = ek * jnp.sin(float(k) * ai)
            keep = rowi >= k
            tab_ref[_TAB_L + 16 * s:_TAB_L + 16 * s + 8, :] = jnp.where(keep, lkr, 0.0)
            tab_ref[_TAB_L + 16 * s + 8:_TAB_L + 16 * s + 16, :] = jnp.where(keep, lki, 0.0)
        kk = rowf + 1.0
        ek = jnp.exp(kk * ar)
        tab_ref[_TAB_P8:_TAB_P8 + 8, :] = ek * jnp.cos(kk * ai)
        tab_ref[_TAB_P8 + 8:_TAB_P8 + 16, :] = ek * jnp.sin(kk * ai)
        car_ref[...] = jnp.zeros_like(car_ref)

    xT = x_ref[...]
    x = xT.T

    wr = _dot_t(x, bre_ref[...])
    wi = _dot_t(x, bim_ref[...])
    qr = tab_ref[_TAB_Q:_TAB_Q + 1, :]
    qi = tab_ref[_TAB_Q + 1:_TAB_Q + 2, :]
    vr = wr * qr - wi * qi
    vi = wr * qi + wi * qr

    gw_col = gw_ref[...].reshape(1, D).T
    prodT = xT * gw_col
    sT = jnp.sum(prodT.astype(_F32), axis=0, keepdims=True)
    sT = _rb(sT)
    gateT = _rb(1.0 / (1.0 + jnp.exp(-sT)))
    omgT = _rb(1.0 - gateT)

    def ffn_slab(j):
        wgs = wg_ref[:, j * FS:(j + 1) * FS]
        wus = wu_ref[:, j * FS:(j + 1) * FS]
        g = _rb(_dot(x, wgs))
        u = _rb(_dot(x, wus))
        gg = jax.nn.gelu(g, approximate=True)
        hf = (gg * u).astype(_BF16)
        wds = wdt_ref[:, j * FS:(j + 1) * FS]
        return _dot_t(wds, hf)

    bT = None
    j = 0

    for s, k in enumerate((1, 2, 4)):
        if j < NSLAB:
            bj = ffn_slab(j)
            bT = bj if bT is None else bT + bj
            j += 1
        lkr = tab_ref[_TAB_L + 16 * s:_TAB_L + 16 * s + 8, :]
        lki = tab_ref[_TAB_L + 16 * s + 8:_TAB_L + 16 * s + 16, :]
        sr3 = pltpu.roll(vr, k, axis=0).reshape(NGRP, _G, P)
        si3 = pltpu.roll(vi, k, axis=0).reshape(NGRP, _G, P)
        vr3 = vr.reshape(NGRP, _G, P)
        vi3 = vi.reshape(NGRP, _G, P)
        vr = (vr3 + lkr[None] * sr3 - lki[None] * si3).reshape(T, P)
        vi = (vi3 + lkr[None] * si3 + lki[None] * sr3).reshape(T, P)

    while j < NSLAB:
        bj = ffn_slab(j)
        bT = bj if bT is None else bT + bj
        j += 1
    bT = _rb(bT)

    p8r = tab_ref[_TAB_P8:_TAB_P8 + 8, :]
    p8i = tab_ref[_TAB_P8 + 8:_TAB_P8 + 16, :]
    cr = car_ref[0:1, :]
    ci = car_ref[8:9, :]
    vr3 = vr.reshape(NGRP, _G, P)
    vi3 = vi.reshape(NGRP, _G, P)
    out_r = []
    out_i = []
    for g in range(NGRP):
        cbr = jnp.broadcast_to(cr, (_G, P))
        cbi = jnp.broadcast_to(ci, (_G, P))
        gr = vr3[g] + (p8r * cbr - p8i * cbi)
        gi = vi3[g] + (p8r * cbi + p8i * cbr)
        out_r.append(gr)
        out_i.append(gi)
        cr = gr[_G - 1:_G, :]
        ci = gi[_G - 1:_G, :]
    car_ref[0:1, :] = cr
    car_ref[8:9, :] = ci
    vr = jnp.concatenate(out_r, axis=0)
    vi = jnp.concatenate(out_i, axis=0)

    yT = (_dot_t(cre_ref[...], vr.astype(_BF16))
          - _dot_t(cim_ref[...], vi.astype(_BF16)))
    dskip_col = dskip_ref[...].reshape(1, D).T
    skipT = (xT * dskip_col).astype(_F32)
    aT = 2.0 * yT + skipT

    o_ref[...] = gateT * aT + _rb(omgT * bT)


@jax.jit
def pallas_gated_mix__ssm_conv_s5__glu_gated_geglu__prompt_kernel(
    A_x: jax.Array,
    A_Lambda_re: jax.Array,
    A_Lambda_im: jax.Array,
    A_B_re: jax.Array,
    A_B_im: jax.Array,
    A_C_re: jax.Array,
    A_C_im: jax.Array,
    A_log_dt: jax.Array,
    A_Dskip: jax.Array,
    B_x: jax.Array,
    B_w_gate: jax.Array,
    B_w_up: jax.Array,
    B_w_down: jax.Array,
    gate_w: jax.Array,
):
    Bsz, L, D = A_x.shape
    P = A_Lambda_re.shape[0]
    F = B_w_gate.shape[1]
    T = 512
    FS = 896
    assert L % T == 0 and F % FS == 0 and T % _G == 0
    nchunks = (Bsz * L) // T

    xT = A_x.reshape(Bsz * L, D).T
    wdt = B_w_down.T

    kernel = functools.partial(_ssm_glu_kernel, T=T, FS=FS)

    def const(shape):
        return pl.BlockSpec(shape, lambda c: tuple(0 for _ in shape))

    outT = pl.pallas_call(
        kernel,
        grid=(nchunks,),
        in_specs=[
            pl.BlockSpec((D, T), lambda c: (0, c)),
            const((D, F)),
            const((D, F)),
            const((D, F)),
            const((P, D)),
            const((P, D)),
            const((D, P)),
            const((D, P)),
            const((P,)),
            const((P,)),
            const((P,)),
            const((D,)),
            const((D,)),
        ],
        out_specs=pl.BlockSpec((D, T), lambda c: (0, c)),
        out_shape=jax.ShapeDtypeStruct((D, Bsz * L), _F32),
        scratch_shapes=[
            pltpu.VMEM((_TAB_ROWS, P), _F32),
            pltpu.VMEM((16, P), _F32),
        ],
        compiler_params=pltpu.CompilerParams(
            dimension_semantics=("arbitrary",),
            vmem_limit_bytes=100 * 1024 * 1024,
        ),
    )(xT, B_w_gate, B_w_up, wdt, A_B_re, A_B_im, A_C_re, A_C_im,
      A_Lambda_re, A_Lambda_im, A_log_dt, A_Dskip, gate_w)
    return outT.T.reshape(Bsz, L, D)
```
